```python
import os as _os
_os.environ.setdefault("JAX_PLATFORMS", "cpu")
import jax
import jax.numpy as jnp

def _softmax(x, axis=-1):
    return jax.nn.softmax(x, axis=axis)
def _gelu(x):
    return jax.nn.gelu(x, approximate=True)
def _silu(x):
    return jax.nn.silu(x)
def _sigmoid(x):
    return jax.nn.sigmoid(x)
def _layernorm(x, axis=-1, eps=1e-5):
    m = jnp.mean(x, axis=axis, keepdims=True)
    v = jnp.var(x, axis=axis, keepdims=True)
    return (x - m) / jnp.sqrt(v + eps)
def _scatter_add(tgt, idx, src, axis=0):
    return tgt.at[idx].add(src)
def _segment_sum(src, seg, n):
    return jax.ops.segment_sum(src, seg, n)
class _Rng:
    def __init__(self, key):
        self._k = key
    def _next(self):
        self._k, sub = jax.random.split(self._k)
        return sub
    def normal(self, shape):
        return jax.random.normal(self._next(), shape, dtype=jnp.bfloat16)
    def randint(self, lo, hi, shape):
        return jax.random.randint(self._next(), shape, lo, hi, dtype=jnp.int32)
    def uniform(self, shape, lo=0.0, hi=1.0):
        return jax.random.uniform(self._next(), shape, jnp.bfloat16, lo, hi)
    def permutation(self, n):
        return jax.random.permutation(self._next(), n)


kernel_name = 'gated_mix__mha_block__mha_block__prompt'

def setup_inputs():
    _rng = _Rng(jax.random.key(int.from_bytes(__import__("os").urandom(4), "little")))
    _w = (lambda a: (lambda t: t.astype(jnp.bfloat16) if jnp.issubdtype(t.dtype, jnp.floating) else t)(jnp.asarray(a)))
    def _A_setup():
        B, S, D, H = 1, 2048, 448, 16
        return {
            "x": _w((lambda *s: _rng.normal(s) * 0.05)(B, S, D)),
            "wqkv": _w((lambda *s: _rng.normal(s) * 0.4)(D, 3 * D)),
            "wo": _w((lambda *s: _rng.normal(s) * 0.05)(D, D)),
        }
    _A_in = _A_setup()

    def _B_setup():
        B, S, D, H = 1, 2048, 448, 16
        return {
            "x": _w((lambda *s: _rng.normal(s) * 0.05)(B, S, D)),
            "wqkv": _w((lambda *s: _rng.normal(s) * 0.4)(D, 3 * D)),
            "wo": _w((lambda *s: _rng.normal(s) * 0.05)(D, D)),
        }
    _B_in = _B_setup()

    return {
        "A_x": _A_in["x"],
        "A_wqkv": _A_in["wqkv"],
        "A_wo": _A_in["wo"],
        "B_x": _B_in["x"],
        "B_wqkv": _B_in["wqkv"],
        "B_wo": _B_in["wo"],
        "gate_w": _w((lambda *s: _rng.normal(s) * 0.05)(448) * 16.0),
    }

def reference(A_x, A_wqkv, A_wo, B_x, B_wqkv, B_wo, gate_w):
    def _A_ref(x, wqkv, wo):
        B, S, D = x.shape
        H = 16
        Dh = D // H
        qkv = (lambda x, *d: x.transpose(*d))((x @ wqkv).reshape(B, S, 3, H, Dh), 2, 0, 3, 1, 4)
        q, k, v = qkv[0], qkv[1], qkv[2]
        scores = jnp.einsum("bhqd,bhkd->bhqk", q, k) * (Dh ** -0.5)
        p = _softmax(scores, axis=-1)
        o = jnp.einsum("bhqk,bhkd->bhqd", p, v)
        return (lambda x, *d: x.transpose(*d))(o, 0, 2, 1, 3).reshape(B, S, D) @ wo

    def _B_ref(x, wqkv, wo):
        B, S, D = x.shape
        H = 16
        Dh = D // H
        qkv = (lambda x, *d: x.transpose(*d))((x @ wqkv).reshape(B, S, 3, H, Dh), 2, 0, 3, 1, 4)
        q, k, v = qkv[0], qkv[1], qkv[2]
        scores = jnp.einsum("bhqd,bhkd->bhqk", q, k) * (Dh ** -0.5)
        p = _softmax(scores, axis=-1)
        o = jnp.einsum("bhqk,bhkd->bhqd", p, v)
        return (lambda x, *d: x.transpose(*d))(o, 0, 2, 1, 3).reshape(B, S, D) @ wo

    x = A_x
    g = _sigmoid((x * gate_w).sum(-1, keepdims=True))
    a = _A_ref(x, A_wqkv, A_wo)
    b = _B_ref(x, B_wqkv, B_wo)
    return g * a + (1 - g) * b
```

```python
import functools
import jax, jax.numpy as jnp, numpy as np
from jax import lax
from jax.experimental import pallas as pl
from jax.experimental.pallas import tpu as pltpu

S, D, H, DH, HP = 2048, 448, 16, 28, 32
DP = H * HP
GW = 4 * DH
BF = jnp.bfloat16
F32 = jnp.float32
QSCALE = float(DH ** -0.5 * np.log2(np.e))
BOUND = 32.0
NT = (((1,), (1,)), ((), ()))

def make(MQ=2048, NK=512, PC=512, EC=512, hun=1, FQ=512, FK=256, check=True, rep=1, kform='TT', hbm=False):
    NC = S // PC
    NE = S // EC
    def kernel(x_hbm, aw_hbm, ao_hbm, bw_hbm, bo_hbm, gw_hbm, out_hbm,
               xv, wv_, wov, gwv, qT, kk, vT, woT, oT, wq_s, wk_s, wv_s, gT, outv, nrm, flag, sems):
        x_cp = [pltpu.make_async_copy(x_hbm.at[:, pl.ds(c * PC, PC)], xv.at[:, pl.ds(c * PC, PC)], sems.at[c]) for c in range(NC)]
        w_cp = [pltpu.make_async_copy(r, wv_.at[m], sems.at[NC + m]) for m, r in enumerate((aw_hbm, bw_hbm))]
        o_cp = [pltpu.make_async_copy(r, wov.at[m], sems.at[NC + 2 + m]) for m, r in enumerate((ao_hbm, bo_hbm))]
        g_cp = pltpu.make_async_copy(gw_hbm, gwv, sems.at[NC + 4])
        w_cp[0].start()
        x_cp[0].start()
        w_cp[0].wait()
        for c in range(1, NC):
            x_cp[c].start()
        w_cp[1].start(); o_cp[0].start(); o_cp[1].start(); g_cp.start()

        zpad = jnp.zeros((HP - DH, D), F32)
        def module(m, _):
            @pl.when(m == 1)
            def _w():
                w_cp[1].wait()
            wt = wv_[m].astype(F32).T
            wq_s[...] = wt[0:D].astype(BF)
            for g in range(4):
                wk_s[128 * g:128 * g + GW, :] = wt[D + GW * g:D + GW * (g + 1)].astype(BF)
                wk_s[128 * g + GW:128 * (g + 1), :] = jnp.zeros((128 - GW, D), BF)
            for j in range(H):
                wv_s[HP * j:HP * (j + 1), :] = jnp.concatenate(
                    [wt[2 * D + DH * j:2 * D + DH * (j + 1)], zpad], axis=0).astype(BF)
            def chunk(c, carry):
                qmax, kmax = carry
                @pl.when(m == 0)
                def _x():
                    pltpu.make_async_copy(x_hbm.at[:, pl.ds(0, PC)], xv.at[:, pl.ds(0, PC)], sems.at[c]).wait()
                r = pl.ds(pl.multiple_of(c * PC, PC), PC)
                xc = xv[:, r]
                q = jnp.dot(wq_s[...], xc, preferred_element_type=F32) * QSCALE
                qT[m, :, r] = q.astype(BF)
                v = jnp.dot(wv_s[...], xc, preferred_element_type=F32)
                row = lax.broadcasted_iota(jnp.int32, v.shape, 0)
                vT[m, :, r] = jnp.where(row % HP == DH, 1.0, v).astype(BF)
                k = lax.dot_general(xc, wk_s[...], (((0,), (1,)), ((), ())), preferred_element_type=F32) if kform == 'TT' else lax.dot_general(xc.T, wk_s[...], NT, preferred_element_type=F32)
                for g in range(4):
                    kk[m, g, r, :] = k[:, 128 * g:128 * (g + 1)].astype(BF)
                if check:
                    qmax = jnp.maximum(qmax, jnp.sum((q * q).reshape(4, GW, PC), axis=1))
                    k2 = k * k
                    kmax = tuple(jnp.maximum(kmax[g], jnp.max(jnp.sum(k2[:, 128 * g:128 * (g + 1)], axis=1, keepdims=True), axis=0, keepdims=True)) for g in range(4))
                return qmax, kmax
            qmax, kmax = lax.fori_loop(0, NC, chunk, (jnp.zeros((4, PC), F32), (jnp.zeros((1, 1), F32),) * 4))
            if check:
                qm = jnp.max(qmax, axis=1, keepdims=True)
                ok = jnp.ones((1, 1), jnp.int32)
                for g in range(4):
                    ok = ok * (qm[g:g + 1] * kmax[g] <= (BOUND / 1.02) ** 2).astype(jnp.int32)
                flag[m] = ok[0, 0]
            pltpu.make_async_copy(ao_hbm, wov.at[m], sems.at[NC + 2 + m]).wait()
            wo = wov[m].astype(F32)
            wop = jnp.concatenate([jnp.concatenate([wo[DH * j:DH * (j + 1)], zpad], axis=0) for j in range(H)], axis=0)
            woT[m] = wop.T.astype(BF)
            return _
        lax.fori_loop(0, 2, module, 0)
        g_cp.wait()
        gl = jnp.dot(jnp.broadcast_to(gwv[...], (16, D)), xv[...], preferred_element_type=F32)
        gT[...] = jax.nn.sigmoid(gl[0:8])

        def load_wq(m, h, qs, n):
            g = h // 4
            qg = qT[m, pl.ds(pl.multiple_of(g * GW, 16), GW), qs]
            row = lax.broadcasted_iota(jnp.int32, qg.shape, 0)
            lo = (h % 4) * DH
            wq = jnp.where((row >= lo) & (row < lo + DH), qg, jnp.zeros_like(qg))
            return jnp.concatenate([wq, jnp.zeros((128 - GW, n), BF)], axis=0)

        def fast_head(mh, qi):
            m = mh // H; h = mh % H; g = h // 4
            qs = pl.ds(pl.multiple_of(qi * MQ, MQ), MQ) if MQ < S else slice(None)
            wq = load_wq(m, h, qs, MQ)
            vr = pl.ds(pl.multiple_of(h * HP, HP), HP)
            acc = jnp.zeros((HP, MQ), F32)
            for c in range(S // NK):
                sT = jnp.dot(kk[m, g, c * NK:(c + 1) * NK, :], wq, preferred_element_type=F32)
                pT = jnp.exp2(sT).astype(BF)
                acc = acc + jnp.dot(vT[m, vr, c * NK:(c + 1) * NK], pT, preferred_element_type=F32)
            oT[m, vr, qs] = (acc * (1.0 / acc[DH:DH + 1, :])).astype(BF)

        def fast_all():
            NQ = S // MQ
            def hbody(t, _):
                for u in range(hun):
                    tt = t * hun + u
                    fast_head(tt % (2 * H), tt // (2 * H))
                return _
            lax.fori_loop(0, rep * NQ * 2 * H // hun, lambda t, c: hbody(t % (NQ * 2 * H // hun), c), 0) if rep > 1 else lax.fori_loop(0, NQ * 2 * H // hun, hbody, 0)

        def slow_all():
            def body(t, _):
                mh = t // (S // FQ); qi = t % (S // FQ)
                m = mh // H; h = mh % H; g = h // 4
                qs = pl.ds(pl.multiple_of(qi * FQ, FQ), FQ)
                wq = load_wq(m, h, qs, FQ)
                vr = pl.ds(pl.multiple_of(h * HP, HP), HP)
                def kv(c, carry):
                    mx, acc = carry
                    ks = pl.ds(pl.multiple_of(c * FK, FK), FK)
                    sT = jnp.dot(kk[m, g, ks, :], wq, preferred_element_type=F32)
                    mn = jnp.maximum(mx, jnp.max(sT, axis=0, keepdims=True))
                    pT = jnp.exp2(sT - mn).astype(BF)
                    acc = acc * jnp.exp2(mx - mn) + jnp.dot(vT[m, vr, ks], pT, preferred_element_type=F32)
                    return mn, acc
                _m, acc = lax.fori_loop(0, S // FK, kv, (jnp.full((1, FQ), -jnp.inf, F32), jnp.zeros((HP, FQ), F32)))
                oT[m, vr, qs] = (acc * (1.0 / acc[DH:DH + 1, :])).astype(BF)
                return _
            lax.fori_loop(0, 2 * H * S // FQ, body, 0)

        if check:
            safe = (flag[0] * flag[1]) == 1
            pl.when(safe)(fast_all)
            pl.when(jnp.logical_not(safe))(slow_all)
        else:
            fast_all()

        def out_cp(e):
            r = pl.ds(pl.multiple_of(e * EC, EC), EC)
            return pltpu.make_async_copy(outv.at[:, r], out_hbm.at[:, r], sems.at[NC + 5 + e])
        def epi(e, _):
            r = pl.ds(pl.multiple_of(e * EC, EC), EC)
            a = jnp.dot(woT[0], oT[0, :, r], preferred_element_type=F32)
            b = jnp.dot(woT[1], oT[1, :, r], preferred_element_type=F32)
            gq = gT[0:1, r]
            res = gq * a + (1.0 - gq) * b
            outv[:, r] = res.astype(BF)
            out_cp(e).start()
            return _
        lax.fori_loop(0, NE, epi, 0)
        for e in range(NE):
            out_cp(e).wait()

    anyspec = pl.BlockSpec(memory_space=pltpu.HBM if hbm else pl.ANY)
    def fn(A_x, A_wqkv, A_wo, B_x, B_wqkv, B_wo, gate_w):
        out = pl.pallas_call(
            kernel,
            in_specs=[anyspec] * 6, out_specs=anyspec,
            out_shape=jax.ShapeDtypeStruct((D, S), BF),
            scratch_shapes=[
                pltpu.VMEM((D, S), BF), pltpu.VMEM((2, D, 3 * D), BF), pltpu.VMEM((2, D, D), BF), pltpu.VMEM((1, D), BF),
                pltpu.VMEM((2, D, S), BF), pltpu.VMEM((2, 4, S, 128), BF), pltpu.VMEM((2, DP, S), BF),
                pltpu.VMEM((2, D, DP), BF), pltpu.VMEM((2, DP, S), BF),
                pltpu.VMEM((D, D), BF), pltpu.VMEM((DP, D), BF), pltpu.VMEM((DP, D), BF),
                pltpu.VMEM((8, S), F32), pltpu.VMEM((D, S), BF), pltpu.VMEM((8, 128), F32),
                pltpu.SMEM((2,), jnp.int32), pltpu.SemaphoreType.DMA((NC + 5 + NE,))],
            compiler_params=pltpu.CompilerParams(vmem_limit_bytes=100 * 2**20),
        )(A_x.reshape(S, D).T, A_wqkv, A_wo, B_wqkv, B_wo, gate_w.reshape(1, D))
        return out.T.reshape(1, S, D)
    return fn


_impl = make(MQ=2048,NK=512)


@jax.jit
def pallas_gated_mix__mha_block__mha_block__prompt_kernel(
    A_x: jax.Array,
    A_wqkv: jax.Array,
    A_wo: jax.Array,
    B_x: jax.Array,
    B_wqkv: jax.Array,
    B_wo: jax.Array,
    gate_w: jax.Array,
):
    return _impl(A_x, A_wqkv, A_wo, B_x, B_wqkv, B_wo, gate_w)
```

```python
import functools
import jax, jax.numpy as jnp, numpy as np
from jax import lax
from jax.experimental import pallas as pl
from jax.experimental.pallas import tpu as pltpu

S, D, H, DH, HP = 2048, 448, 16, 28, 32
DP = H * HP
GW = 4 * DH
BF = jnp.bfloat16
F32 = jnp.float32
QSCALE = float(DH ** -0.5 * np.log2(np.e))
BOUND = 32.0
NT = (((1,), (1,)), ((), ()))

def make(MQ=2048, NK=512, PC=512, EC=512, hun=1, FQ=512, FK=256, check=True, rep=1, kform='TT', hbm=False, flags=None, prep=1, PS=1, kT16=True, kpad=True):
    NC = S // PC
    NE = S // EC
    def kernel(x_hbm, aw_hbm, ao_hbm, bw_hbm, bo_hbm, gw_hbm, out_hbm,
               xv, wv_, wov, gwv, qT, kk, vT, woT, oT, wq_s, wk_s, wv_s, gT, outv, nrm, flag, sems):
        x_cp = [pltpu.make_async_copy(x_hbm.at[:, pl.ds(c * PC, PC)], xv.at[:, pl.ds(c * PC, PC)], sems.at[c]) for c in range(NC)]
        w_cp = [pltpu.make_async_copy(r, wv_.at[m], sems.at[NC + m]) for m, r in enumerate((aw_hbm, bw_hbm))]
        o_cp = [pltpu.make_async_copy(r, wov.at[m], sems.at[NC + 2 + m]) for m, r in enumerate((ao_hbm, bo_hbm))]
        g_cp = pltpu.make_async_copy(gw_hbm, gwv, sems.at[NC + 4])
        g_cp.start()
        w_cp[0].start()
        x_cp[0].start()
        wov[2] = jnp.zeros((D, D), BF)
        w_cp[0].wait()
        for c in range(1, NC):
            x_cp[c].start()
        w_cp[1].start(); o_cp[0].start(); o_cp[1].start()

        zpad = jnp.zeros((HP - DH, D), F32)
        g_cp.wait()
        gcol = jnp.broadcast_to(gwv[...].reshape(1, D).astype(F32), (128, D)).T
        HC = H // NC
        def module(m, carry0):
            @pl.when(m == 1)
            def _w():
                w_cp[1].wait()
                o_cp[0].wait()
                o_cp[1].wait()
            def chunk(c, carry):
                qmax, kmax = carry
                @pl.when(m == 0)
                def _x():
                    pltpu.make_async_copy(x_hbm.at[:, pl.ds(0, PC)], xv.at[:, pl.ds(0, PC)], sems.at[c]).wait()
                PS_ = PC // PS
                assert NC == 2
                sl = jnp.where(m == 1, c, 2)
                wo = wov[sl].astype(F32)
                wop = jnp.concatenate([jnp.concatenate([wo[DH * j:DH * (j + 1)], zpad], axis=0) for j in range(H)], axis=0)
                woT[sl] = wop.T.astype(BF)
                for sb in range(PS):
                    r = pl.ds(pl.multiple_of(c * PC + sb * PS_, PS_), PS_)
                    xc = xv[:, r]
                    y = lax.dot_general(wv_[m], xc, (((0,), (0,)), ((), ())), preferred_element_type=F32)
                    xf = xc.astype(F32)
                    gl = jnp.concatenate([jnp.sum(xf[:, t * 128:(t + 1) * 128] * gcol, axis=0, keepdims=True) for t in range(PS_ // 128)], axis=1)
                    gT[0:1, r] = jax.nn.sigmoid(gl)
                    q = y[0:D] * QSCALE
                    qT[m, :, r] = q.astype(BF)
                    zrow = jnp.zeros((128 - GW, PS_), F32)
                    for g in range(4):
                        k0 = D + GW * g
                        kg = y[k0:k0 + 128] if (kpad and g < 3) else jnp.concatenate([y[k0:k0 + GW], zrow], axis=0)
                        kk[m, g, r, :] = kg.astype(BF).T if kT16 else kg.T.astype(BF)
                    one = jnp.where(lax.broadcasted_iota(jnp.int32, (HP - DH, PS_), 0) == 0, 1.0, 0.0).astype(F32)
                    for j in range(H):
                        v0 = 2 * D + DH * j
                        vT[m, HP * j:HP * (j + 1), r] = jnp.concatenate([y[v0:v0 + DH], one], axis=0).astype(BF)
                    if check:
                        qmax = jnp.maximum(qmax, jnp.sum((q * q).reshape(4, GW, PS_), axis=1))
                        kf = y[D:2 * D]
                        kmax = jnp.maximum(kmax, jnp.sum((kf * kf).reshape(4, GW, PS_), axis=1))
                return qmax, kmax
            z = jnp.zeros((4, PC // PS), F32)
            qmax, kmax = lax.fori_loop(0, NC, chunk, (z, z))
            if check:
                nrm[m, 0:4, :] = qmax
                nrm[m, 4:8, :] = kmax
            return carry0
        lax.fori_loop(0, 2, module, 0)
        if check:
            mx = jnp.max(nrm[...].reshape(16, PC // PS), axis=1, keepdims=True)
            bnd = jnp.concatenate([mx[0:4] * mx[4:8], mx[8:12] * mx[12:16]], axis=0)
            ok = jnp.min((bnd <= (BOUND / 1.02) ** 2).astype(jnp.int32), axis=0, keepdims=True)
            flag[0] = ok[0, 0]

        def load_wq(m, h, qs, n):
            g = h // 4
            qg = qT[m, pl.ds(pl.multiple_of(g * GW, 16), GW), qs]
            row = lax.broadcasted_iota(jnp.int32, qg.shape, 0)
            lo = (h % 4) * DH
            wq = jnp.where((row >= lo) & (row < lo + DH), qg, jnp.zeros_like(qg))
            return jnp.concatenate([wq, jnp.zeros((128 - GW, n), BF)], axis=0)

        def fast_head(mh, qi):
            m = mh // H; h = mh % H; g = h // 4
            qs = pl.ds(pl.multiple_of(qi * MQ, MQ), MQ) if MQ < S else slice(None)
            wq = load_wq(m, h, qs, MQ)
            vr = pl.ds(pl.multiple_of(h * HP, HP), HP)
            acc = jnp.zeros((HP, MQ), F32)
            for c in range(S // NK):
                sT = jnp.dot(kk[m, g, c * NK:(c + 1) * NK, :], wq, preferred_element_type=F32)
                pT = jnp.exp2(sT).astype(BF)
                acc = acc + jnp.dot(vT[m, vr, c * NK:(c + 1) * NK], pT, preferred_element_type=F32)
            oT[m, vr, qs] = (acc * (1.0 / acc[DH:DH + 1, :])).astype(BF)

        def fast_all():
            NQ = S // MQ
            def hbody(t, _):
                for u in range(hun):
                    tt = t * hun + u
                    fast_head(tt % (2 * H), tt // (2 * H))
                return _
            lax.fori_loop(0, rep * NQ * 2 * H // hun, lambda t, c: hbody(t % (NQ * 2 * H // hun), c), 0) if rep > 1 else lax.fori_loop(0, NQ * 2 * H // hun, hbody, 0)

        def slow_all():
            def body(t, _):
                mh = t // (S // FQ); qi = t % (S // FQ)
                m = mh // H; h = mh % H; g = h // 4
                qs = pl.ds(pl.multiple_of(qi * FQ, FQ), FQ)
                wq = load_wq(m, h, qs, FQ)
                vr = pl.ds(pl.multiple_of(h * HP, HP), HP)
                def kv(c, carry):
                    mx, acc = carry
                    ks = pl.ds(pl.multiple_of(c * FK, FK), FK)
                    sT = jnp.dot(kk[m, g, ks, :], wq, preferred_element_type=F32)
                    mn = jnp.maximum(mx, jnp.max(sT, axis=0, keepdims=True))
                    pT = jnp.exp2(sT - mn).astype(BF)
                    acc = acc * jnp.exp2(mx - mn) + jnp.dot(vT[m, vr, ks], pT, preferred_element_type=F32)
                    return mn, acc
                _m, acc = lax.fori_loop(0, S // FK, kv, (jnp.full((1, FQ), -jnp.inf, F32), jnp.zeros((HP, FQ), F32)))
                oT[m, vr, qs] = (acc * (1.0 / acc[DH:DH + 1, :])).astype(BF)
                return _
            lax.fori_loop(0, 2 * H * S // FQ, body, 0)

        if check:
            safe = flag[0] == 1
            pl.when(safe)(fast_all)
            pl.when(jnp.logical_not(safe))(slow_all)
        else:
            fast_all()

        def out_cp(e):
            r = pl.ds(pl.multiple_of(e * EC, EC), EC)
            return pltpu.make_async_copy(outv.at[:, r], out_hbm.at[:, r], sems.at[NC + 5 + e])
        def epi(e, _):
            r = pl.ds(pl.multiple_of(e * EC, EC), EC)
            a = jnp.dot(woT[0], oT[0, :, r], preferred_element_type=F32)
            b = jnp.dot(woT[1], oT[1, :, r], preferred_element_type=F32)
            gq = gT[0:1, r]
            res = gq * a + (1.0 - gq) * b
            outv[:, r] = res.astype(BF)
            out_cp(e).start()
            return _
        lax.fori_loop(0, NE, epi, 0)
        for e in range(NE):
            out_cp(e).wait()

    anyspec = pl.BlockSpec(memory_space=pltpu.HBM if hbm else pl.ANY)
    def fn(A_x, A_wqkv, A_wo, B_x, B_wqkv, B_wo, gate_w):
        out = pl.pallas_call(
            kernel,
            in_specs=[anyspec] * 6, out_specs=anyspec,
            out_shape=jax.ShapeDtypeStruct((D, S), BF),
            scratch_shapes=[
                pltpu.VMEM((D, S), BF), pltpu.VMEM((2, D, 3 * D), BF), pltpu.VMEM((3, D, D), BF), pltpu.VMEM((D,), BF),
                pltpu.VMEM((2, D, S), BF), pltpu.VMEM((2, 4, S, 128), BF), pltpu.VMEM((2, DP, S), BF),
                pltpu.VMEM((3, D, DP), BF), pltpu.VMEM((2, DP, S), BF),
                pltpu.VMEM((D, D), BF), pltpu.VMEM((DP, D), BF), pltpu.VMEM((DP, D), BF),
                pltpu.VMEM((8, S), F32), pltpu.VMEM((D, S), BF), pltpu.VMEM((2, 8, PC // PS), F32),
                pltpu.SMEM((2,), jnp.int32), pltpu.SemaphoreType.DMA((NC + 5 + NE,))],
            compiler_params=pltpu.CompilerParams(vmem_limit_bytes=100 * 2**20, flags=flags),
        )(A_x.reshape(S, D).T, A_wqkv, A_wo, B_wqkv, B_wo, gate_w)
        return out.T.reshape(1, S, D)
    return fn


_impl = make(MQ=2048,NK=512,PC=1024,PS=2,hun=4)


@jax.jit
def pallas_gated_mix__mha_block__mha_block__prompt_kernel(
    A_x: jax.Array,
    A_wqkv: jax.Array,
    A_wo: jax.Array,
    B_x: jax.Array,
    B_wqkv: jax.Array,
    B_wo: jax.Array,
    gate_w: jax.Array,
):
    return _impl(A_x, A_wqkv, A_wo, B_x, B_wqkv, B_wo, gate_w)
```

```python
import jax
import jax.numpy as jnp
import numpy as np
from jax import lax
from jax.experimental import pallas as pl
from jax.experimental.pallas import tpu as pltpu

S, D, H, DH = 2048, 448, 16, 28
HP = 32
GW = 4 * DH
PC, PS = 1024, 512
NK = 512
HUN = 4
EC = 512
FK = 512
NC, NE = S // PC, S // EC
BF, F32 = jnp.bfloat16, jnp.float32
QSCALE = float(DH ** -0.5 * np.log2(np.e))
BOUND = 48.0


def _kernel(x_hbm, aw_hbm, ao_hbm, bw_hbm, bo_hbm, gw_hbm, out_hbm,
            xv, wv, wT, wov, woT, gwv, gT, qT, kk, vT, oT, outv, nrm, flag, sems):
    def x_cp(c):
        r = pl.ds(pl.multiple_of(c * PC, PC), PC)
        return pltpu.make_async_copy(x_hbm.at[:, r], xv.at[:, r], sems.at[c])

    def out_cp(e):
        r = pl.ds(pl.multiple_of(e * EC, EC), EC)
        return pltpu.make_async_copy(outv.at[:, r], out_hbm.at[:, r], sems.at[NC + 5 + e])

    w_cp = [pltpu.make_async_copy(r, wv.at[m], sems.at[NC + m])
            for m, r in enumerate((aw_hbm, bw_hbm))]
    o_cp = [pltpu.make_async_copy(r, wov.at[pl.ds(m * D, D), :], sems.at[NC + 2 + m])
            for m, r in enumerate((ao_hbm, bo_hbm))]
    g_cp = pltpu.make_async_copy(gw_hbm, gwv, sems.at[NC + 4])

    g_cp.start()
    w_cp[0].start()
    x_cp(0).start()
    wov[2 * D:2 * D + 512, :] = jnp.zeros((512, D), BF)
    w_cp[0].wait()
    for c in range(1, NC):
        x_cp(c).start()
    w_cp[1].start()
    o_cp[0].start()
    o_cp[1].start()
    g_cp.wait()
    gcol = jnp.broadcast_to(gwv[...].reshape(1, D).astype(F32), (128, D)).T
    wT[0] = wv[0].T

    def module(m, carry0):
        @pl.when(m == 1)
        def _():
            o_cp[0].wait()
            o_cp[1].wait()

        def chunk(c, carry):
            qmax, kmax = carry

            @pl.when(m == 0)
            def _():
                x_cp(c).wait()

            nxt = jnp.logical_and(m == 0, c == 1)

            @pl.when(nxt)
            def _():
                w_cp[1].wait()

            ro = pl.multiple_of(jnp.where(m == 1, c * 384, 2 * D), 128)
            woT[:, pl.ds(ro, 512)] = wov[pl.ds(ro, 512), :].T
            rg = pl.ds(pl.multiple_of(c * PC + m * PS, PS), PS)
            xf = xv[:, rg].astype(F32)
            gl = jnp.concatenate(
                [jnp.sum(xf[:, t * 128:(t + 1) * 128] * gcol, axis=0, keepdims=True)
                 for t in range(PS // 128)], axis=1)
            gT[0:1, rg] = jax.nn.sigmoid(gl)

            for sb in range(PC // PS):
                r = pl.ds(pl.multiple_of(c * PC + sb * PS, PS), PS)
                y = jnp.dot(wT[m], xv[:, r], preferred_element_type=F32)
                q = y[0:D] * QSCALE
                qT[m, :, r] = q.astype(BF)
                for g in range(4):
                    k0 = D + GW * g
                    kg = (y[k0:k0 + 128] if g < 3 else
                          jnp.concatenate([y[k0:k0 + GW], jnp.zeros((128 - GW, PS), F32)], axis=0))
                    kk[m, g, r, :] = kg.astype(BF).T
                one = jnp.where(lax.broadcasted_iota(jnp.int32, (HP - DH, PS), 0) == 0,
                                1.0, 0.0).astype(F32)
                for j in range(H):
                    v0 = 2 * D + DH * j
                    vT[m, HP * j:HP * (j + 1), r] = jnp.concatenate(
                        [y[v0:v0 + DH], one], axis=0).astype(BF)
                kf = y[D:2 * D]
                qmax = jnp.maximum(qmax, jnp.sum((q * q).reshape(8, GW // 2, PS), axis=1))
                kmax = jnp.maximum(kmax, jnp.sum((kf * kf).reshape(8, GW // 2, PS), axis=1))
            wT[jnp.where(nxt, 1, 2)] = wv[jnp.where(nxt, 1, 0)].T
            return qmax, kmax

        z = jnp.zeros((8, PS), F32)
        qmax, kmax = lax.fori_loop(0, NC, chunk, (z, z))
        nrm[m, 0] = qmax
        nrm[m, 1] = kmax
        return carry0

    lax.fori_loop(0, 2, module, 0)

    mq = jnp.max(nrm[:, 0].reshape(16, PS), axis=1, keepdims=True)
    mk = jnp.max(nrm[:, 1].reshape(16, PS), axis=1, keepdims=True)
    ok = jnp.min((mq * mk <= (BOUND / 1.02) ** 2).astype(jnp.int32), axis=0, keepdims=True)
    flag[0] = ok[0, 0]

    def load_wq(m, h):
        qg = qT[m, pl.ds(pl.multiple_of((h // 4) * GW, 16), GW), :]
        row = lax.broadcasted_iota(jnp.int32, qg.shape, 0)
        lo = (h % 4) * DH
        wq = jnp.where((row >= lo) & (row < lo + DH), qg, jnp.zeros_like(qg))
        return jnp.concatenate([wq, jnp.zeros((128 - GW, S), BF)], axis=0)

    def store_head(mh, acc):
        gq = gT[0:1, :]
        sc = jnp.where(mh < H, gq, 1.0 - gq) / acc[DH:DH + 1, :]
        oT[mh] = (acc * sc).astype(BF)

    def fast_head(mh):
        m, h = mh // H, mh % H
        wq = load_wq(m, h)
        vr = pl.ds(pl.multiple_of(h * HP, HP), HP)
        acc = jnp.zeros((HP, S), F32)
        for c in range(S // NK):
            ks = slice(c * NK, (c + 1) * NK)
            sT = jnp.dot(kk[m, h // 4, ks, :], wq, preferred_element_type=F32)
            pT = jnp.exp2(sT).astype(BF)
            acc = acc + jnp.dot(vT[m, vr, ks], pT, preferred_element_type=F32)
        store_head(mh, acc)

    def fast_all():
        def body(t, carry):
            for u in range(HUN):
                fast_head(t * HUN + u)
            return carry
        lax.fori_loop(0, 2 * H // HUN, body, 0)

    def safe_all():
        def body(mh, carry):
            m, h = mh // H, mh % H
            wq = load_wq(m, h)
            vr = pl.ds(pl.multiple_of(h * HP, HP), HP)

            def kv(c, st):
                mx, acc = st
                ks = pl.ds(pl.multiple_of(c * FK, FK), FK)
                sT = jnp.dot(kk[m, h // 4, ks, :], wq, preferred_element_type=F32)
                mn = jnp.maximum(mx, jnp.max(sT, axis=0, keepdims=True))
                pT = jnp.exp2(sT - mn).astype(BF)
                acc = acc * jnp.exp2(mx - mn) + jnp.dot(vT[m, vr, ks], pT,
                                                        preferred_element_type=F32)
                return mn, acc

            _, acc = lax.fori_loop(0, S // FK, kv, (jnp.full((1, S), -jnp.inf, F32),
                                                    jnp.zeros((HP, S), F32)))
            store_head(mh, acc)
            return carry
        lax.fori_loop(0, 2 * H, body, 0)

    safe = flag[0] == 1
    pl.when(safe)(fast_all)
    pl.when(jnp.logical_not(safe))(safe_all)

    def epi(e, carry):
        r = pl.ds(pl.multiple_of(e * EC, EC), EC)
        oc = jnp.concatenate([oT[j, :, r].astype(F32)[0:DH] for j in range(2 * H)],
                             axis=0).astype(BF)
        res = jnp.dot(woT[:, 0:2 * D], oc, preferred_element_type=F32)
        outv[:, r] = res.astype(BF)
        out_cp(e).start()
        return carry

    lax.fori_loop(0, NE, epi, 0)
    for e in range(NE):
        out_cp(e).wait()


@jax.jit
def pallas_gated_mix__mha_block__mha_block__prompt_kernel(
    A_x: jax.Array,
    A_wqkv: jax.Array,
    A_wo: jax.Array,
    B_x: jax.Array,
    B_wqkv: jax.Array,
    B_wo: jax.Array,
    gate_w: jax.Array,
):
    hbm = pl.BlockSpec(memory_space=pl.ANY)
    out_t = pl.pallas_call(
        _kernel,
        in_specs=[hbm] * 6,
        out_specs=hbm,
        out_shape=jax.ShapeDtypeStruct((D, S), BF),
        scratch_shapes=[
            pltpu.VMEM((D, S), BF),
            pltpu.VMEM((2, D, 3 * D), BF),
            pltpu.VMEM((3, 3 * D, D), BF),
            pltpu.VMEM((2 * D + 512, D), BF),
            pltpu.VMEM((D, 2 * D + 512), BF),
            pltpu.VMEM((D,), BF),
            pltpu.VMEM((8, S), F32),
            pltpu.VMEM((2, D, S), BF),
            pltpu.VMEM((2, 4, S, 128), BF),
            pltpu.VMEM((2, H * HP, S), BF),
            pltpu.VMEM((2 * H, HP, S), BF),
            pltpu.VMEM((D, S), BF),
            pltpu.VMEM((2, 2, 8, PS), F32),
            pltpu.SMEM((1,), jnp.int32),
            pltpu.SemaphoreType.DMA((NC + 5 + NE,)),
        ],
        compiler_params=pltpu.CompilerParams(vmem_limit_bytes=100 * 2**20),
    )(A_x.reshape(S, D).T, A_wqkv, A_wo, B_wqkv, B_wo, gate_w)
    return out_t.T.reshape(1, S, D)
```
